```python
import os as _os
_os.environ.setdefault("JAX_PLATFORMS", "cpu")
import jax
import jax.numpy as jnp

def _softmax(x, axis=-1):
    return jax.nn.softmax(x, axis=axis)
def _gelu(x):
    return jax.nn.gelu(x, approximate=True)
def _silu(x):
    return jax.nn.silu(x)
def _sigmoid(x):
    return jax.nn.sigmoid(x)
def _layernorm(x, axis=-1, eps=1e-5):
    m = jnp.mean(x, axis=axis, keepdims=True)
    v = jnp.var(x, axis=axis, keepdims=True)
    return (x - m) / jnp.sqrt(v + eps)
def _scatter_add(tgt, idx, src, axis=0):
    return tgt.at[idx].add(src)
def _segment_sum(src, seg, n):
    return jax.ops.segment_sum(src, seg, n)
class _Rng:
    def __init__(self, key):
        self._k = key
    def _next(self):
        self._k, sub = jax.random.split(self._k)
        return sub
    def normal(self, shape):
        return jax.random.normal(self._next(), shape, dtype=jnp.bfloat16)
    def randint(self, lo, hi, shape):
        return jax.random.randint(self._next(), shape, lo, hi, dtype=jnp.int32)
    def uniform(self, shape, lo=0.0, hi=1.0):
        return jax.random.uniform(self._next(), shape, jnp.bfloat16, lo, hi)
    def permutation(self, n):
        return jax.random.permutation(self._next(), n)


kernel_name = 'gated_mix__sliding_block__sliding_local_dilated__prompt'

def setup_inputs():
    _rng = _Rng(jax.random.key(int.from_bytes(__import__("os").urandom(4), "little")))
    _w = (lambda a: (lambda t: t.astype(jnp.bfloat16) if jnp.issubdtype(t.dtype, jnp.floating) else t)(jnp.asarray(a)))
    def _A_setup():
        B, S, D = 1, 2048, 640
        return {
            "x": _w((lambda *s: _rng.normal(s) * 0.05)(B, S, D)),
            "wqkv": _w((lambda *s: _rng.normal(s) * 0.8)(D, 3 * D)),
            "wo": _w((lambda *s: _rng.normal(s) * 0.05)(D, D)),
        }
    _A_in = _A_setup()

    def _B_setup():
        B, S, D = 1, 2048, 640
        return {
            "x": _w((lambda *s: _rng.normal(s) * 0.05)(B, S, D)),
            "wqkv": _w((lambda *s: _rng.normal(s) * 0.8)(D, 3 * D)),
            "wo": _w((lambda *s: _rng.normal(s) * 0.05)(D, D)),
        }
    _B_in = _B_setup()

    return {
        "A_x": _A_in["x"],
        "A_wqkv": _A_in["wqkv"],
        "A_wo": _A_in["wo"],
        "B_x": _B_in["x"],
        "B_wqkv": _B_in["wqkv"],
        "B_wo": _B_in["wo"],
        "gate_w": _w((lambda *s: _rng.normal(s) * 0.05)(640) * 16.0),
    }

def reference(A_x, A_wqkv, A_wo, B_x, B_wqkv, B_wo, gate_w):
    def _A_ref(x, wqkv, wo):
        B, S, D = x.shape
        H = 32; Dh = D // H; W = 256
        qkv = (lambda x, *d: x.transpose(*d))((x @ wqkv).reshape(B, S, 3, H, Dh), 2, 0, 3, 1, 4)
        q, k, v = qkv[0], qkv[1], qkv[2]
        scores = jnp.einsum("bhqd,bhkd->bhqk", q, k) * (Dh ** -0.5)
        idx = jnp.arange(S)
        mask = (idx[:, None] - idx[None, :] >= 0) & (idx[:, None] - idx[None, :] < W)
        scores = jnp.where(mask[None, None], scores, -1e9)
        p = _softmax(scores, axis=-1)
        o = jnp.einsum("bhqk,bhkd->bhqd", p, v)
        return (lambda x, *d: x.transpose(*d))(o, 0, 2, 1, 3).reshape(B, S, D) @ wo

    def _B_ref(x, wqkv, wo):
        B, S, D = x.shape
        H = 32; Dh = D // H
        W, dil = 8, 2
        qkv = (lambda x, *d: x.transpose(*d))((x @ wqkv).reshape(B, S, 3, H, Dh), 2, 0, 3, 1, 4)
        q, k, v = qkv[0], qkv[1], qkv[2]
        scale = Dh ** -0.5
        pos = jnp.arange(S)
        off = jnp.arange(W) * dil
        idx = pos[:, None] - off[None, :]
        mask = idx >= 0
        idx_c = jnp.where(mask, idx, 0).reshape(-1)
        kg = k[:, :, idx_c, :].reshape(B, H, S, W, Dh)
        vg = v[:, :, idx_c, :].reshape(B, H, S, W, Dh)
        logits = jnp.einsum("bhsd,bhswd->bhsw", q, kg) * scale
        logits = jnp.where(mask[None, None, :, :], logits, -1e9)
        attn = _softmax(logits, axis=-1)
        o = jnp.einsum("bhsw,bhswd->bhsd", attn, vg)
        return (lambda x, *d: x.transpose(*d))(o, 0, 2, 1, 3).reshape(B, S, D) @ wo

    x = A_x
    g = _sigmoid((x * gate_w).sum(-1, keepdims=True))
    a = _A_ref(x, A_wqkv, A_wo)
    b = _B_ref(x, B_wqkv, B_wo)
    return g * a + (1 - g) * b
```

```python
import functools
import math

import jax
import jax.numpy as jnp
from jax import lax
import jax.experimental.pallas as pl
import jax.experimental.pallas.tpu as pltpu

S, D, H, DH = 2048, 640, 32, 20
BQ = 256
NT = D // 128
NEG = -1e9
QSCALE = (DH ** -0.5) * math.log2(math.e)
PADB = 16


BCH = 16
NS = 2
G = H // 4


def _win(g):
    return 64 * ((4 * DH * g) // 64) if g < G - 1 else D - 128


def _u32(x):
    return pltpu.bitcast(x, jnp.uint32)


def _bf(x):
    return pltpu.bitcast(x, jnp.bfloat16)


def _recip(x):
    r = pl.reciprocal(x, approx=True)
    return r * (2.0 - x * r)


def _qk(g, nk, qb, q0, ka_ref, qa_ref, s_ref, slot):
    qt = qa_ref[g, qb * 128:(qb + 1) * 128, :]
    lane = lax.broadcasted_iota(jnp.int32, (128, 128), 1)
    qs = []
    for hh in range(4):
        off = DH * (4 * g + hh) - _win(g)
        qs.append(jnp.where((lane >= off) & (lane < off + DH), qt, 0.0))
    qstack = jnp.concatenate(qs, axis=0).astype(jnp.bfloat16)
    kt = ka_ref[g, pl.ds(pl.multiple_of(q0 - 128 * (nk - 1), 128), 128 * nk), :]
    s_ref[slot, 0:128 * nk, :] = lax.dot_general(
        kt, qstack, (((1,), (1,)), ((), ())), preferred_element_type=jnp.float32)


def _softmax(hh, nk, s_ref, p_ref, slot, upper, umask):
    c = slice(128 * hh, 128 * hh + 128)
    ld = lambda n: s_ref[slot, 128 * n:128 * n + 128, c]
    if nk == 3:
        sm = jnp.where(upper, ld(0), ld(2)); s1 = ld(1)
    elif nk == 2:
        sm = jnp.where(upper, NEG, ld(1)); s1 = ld(0)
    else:
        sm = jnp.where(upper, NEG, ld(0)); s1 = None
    mx = jnp.max(sm if s1 is None else jnp.maximum(sm, s1), axis=0, keepdims=True)
    pm = jnp.exp2(sm - mx)
    if nk == 3:
        p_ref[slot, 0:128, c] = jnp.where(upper, pm, 0.0).astype(jnp.bfloat16)
    if nk >= 2:
        p_ref[slot, 128 * (nk - 2):128 * (nk - 1), c] = jnp.exp2(s1 - mx).astype(jnp.bfloat16)
    p_ref[slot, 128 * (nk - 1):128 * nk, c] = (jnp.where(upper, 0.0, pm) if nk == 3 else pm).astype(jnp.bfloat16)


def _pv(g, hh, nk, q0, vs_ref, p_ref, ot_ref, slot):
    h = 4 * g + hh
    ro = (DH * h) % 16
    r1 = (ro + DH) % 32
    kt0 = (q0 // 128) - (nk - 1)
    slabs = [vs_ref[kt0 + n, h] for n in range(nk)]
    vs = jnp.concatenate(slabs, axis=1) if nk > 1 else slabs[0]
    ot = jnp.dot(vs, p_ref[slot, 0:128 * nk, 128 * hh:128 * hh + 128], preferred_element_type=jnp.float32)
    ot_ref[DH * h:DH * h + DH, :] = (ot * _recip(ot[r1:r1 + 1, :]))[ro:ro + DH, :]


def _attn_b_chunk(r0, nr, base, first, qb_ref, kb_ref, vb_ref, ob_ref):
    hs = PADB + base + r0
    q = [qb_ref[t, r0:r0 + nr, :] for t in range(NT)]
    logits = []
    for w in range(8):
        pr = [q[t] * kb_ref[t, pl.ds(hs - 2 * w, nr), :] for t in range(NT)]
        logits.append((pr[0] + pr[1]) + (pr[2] + pr[3]) + pr[4])
    lg = jnp.concatenate(logits, axis=0)
    lg = lg + pltpu.roll(lg, 64, 1)
    lg = lg + pltpu.roll(lg, 32, 1)
    logits = [lg[w * nr:(w + 1) * nr] for w in range(8)]
    if first and r0 < 14:
        pos = lax.broadcasted_iota(jnp.int32, (nr, 128), 0) + r0
        logits = [jnp.where(pos >= 2 * w, l, NEG) if w else l for w, l in enumerate(logits)]
    mx = functools.reduce(jnp.maximum, logits)
    es = [jnp.exp2(l - mx) for l in logits]
    inv = _recip(functools.reduce(jnp.add, es))
    ps = [e * inv for e in es]
    for t in range(NT):
        pr = [ps[w] * vb_ref[t, pl.ds(hs - 2 * w, nr), :] for w in range(8)]
        acc = ((pr[0] + pr[1]) + (pr[2] + pr[3])) + ((pr[4] + pr[5]) + (pr[6] + pr[7]))
        ob_ref[r0:r0 + nr, 128 * t:128 * (t + 1)] = acc.astype(jnp.bfloat16)


def _kernel(xa_ref, wa_hbm, wb_hbm, woa_hbm, wob_hbm, g_ref, o_ref,
            ka_ref, qa_ref, vs_ref, s_ref, p_ref, ot_ref, oa_ref, qb_ref, kb_ref, vb_ref, ob_ref,
            wbt_ref, wop_ref, tmp_ref, acc_ref, wa_ref, wb_ref, woa_ref, wob_ref, sems):
    i = pl.program_id(0)
    base = pl.multiple_of(i * BQ, BQ)

    cp_b = [pltpu.make_async_copy(wb_hbm.at[:, pl.ds(p * D, D)], wb_ref.at[p], sems.at[p]) for p in range(3)]
    cp_a = [pltpu.make_async_copy(wa_hbm.at[:, pl.ds(p * D, D)], wa_ref.at[p], sems.at[3 + p]) for p in range(3)]
    cp_oa = pltpu.make_async_copy(woa_hbm, woa_ref, sems.at[6])
    cp_ob = pltpu.make_async_copy(wob_hbm, wob_ref, sems.at[7])

    def permute_rows(val, dst_ref, r0):
        for t in range(NT):
            tmp_ref[t] = val[:, 128 * t:128 * (t + 1)]
        for d in range(DH):
            for t in range(NT):
                dst_ref[r0 + H * d:r0 + H * d + H, 128 * t:128 * (t + 1)] = (
                    tmp_ref[t, pl.ds(d, H, stride=DH), :].astype(jnp.bfloat16))

    @pl.when(i == 0)
    def _():
        kb_ref[:, 0:PADB, :] = jnp.zeros((NT, PADB, 128), jnp.float32)
        vb_ref[:, 0:PADB, :] = jnp.zeros((NT, PADB, 128), jnp.float32)
        for c in cp_a:
            c.start()
        for c in cp_b:
            c.start()
        cp_ob.start()
        cp_oa.start()

    xa = xa_ref[...]
    nt = (((1,), (1,)), ((), ()))
    def bproj():
        qkvb = lax.dot_general(xa, wbt_ref[...], nt, preferred_element_type=jnp.float32)
        for t in range(NT):
            qb_ref[t] = qkvb[:, 128 * t:128 * (t + 1)] * QSCALE
            kb_ref[t, pl.ds(PADB + base, BQ), :] = qkvb[:, D + 128 * t:D + 128 * (t + 1)]
            vb_ref[t, pl.ds(PADB + base, BQ), :] = qkvb[:, 2 * D + 128 * t:2 * D + 128 * (t + 1)]

    upper = lax.broadcasted_iota(jnp.int32, (128, 128), 0) > lax.broadcasted_iota(jnp.int32, (128, 128), 1)
    umask = None

    def body(first):
        nb = BQ // BCH
        def bchunks(lo, hi):
            for c in range(lo, hi):
                _attn_b_chunk(c * BCH, BCH, base, first, qb_ref, kb_ref, vb_ref, ob_ref)
        if first:
            cp_a[0].wait()
        else:
            bproj()
        gate = jax.nn.sigmoid(jnp.sum(xa.astype(jnp.float32) * g_ref[...].astype(jnp.float32),
                                      axis=1, keepdims=True))
        def oprojb(hf):
            r = slice(hf * 128, (hf + 1) * 128)
            acc_ref[r, :] = (1.0 - gate[r]) * jnp.dot(ob_ref[r, :], wop_ref[...], preferred_element_type=jnp.float32)
        q = jnp.dot(xa, wa_ref[0], preferred_element_type=jnp.float32) * QSCALE
        for g in range(G):
            qa_ref[g] = q[:, _win(g):_win(g) + 128]
        if not first:
            bchunks(0, nb // 2)
            oprojb(0)
        if first:
            cp_a[1].wait()
        k = jnp.dot(xa, wa_ref[1], preferred_element_type=jnp.float32).astype(jnp.bfloat16)
        for g in range(G):
            ka_ref[g, pl.ds(base, BQ), :] = k[:, _win(g):_win(g) + 128]
        if not first:
            bchunks(nb // 2, nb)
            oprojb(1)
        if first:
            cp_a[2].wait()
        vT = jnp.dot(xa, wa_ref[2], preferred_element_type=jnp.float32).T
        row = lax.broadcasted_iota(jnp.int32, (32, 256), 0)
        for h in range(H):
            a = (DH * h) // 16 * 16
            r1 = (DH * h - a + DH) % 32
            slab = jnp.where(row == r1, 1.0, vT[a:a + 32, :]).astype(jnp.bfloat16)
            vs_ref[2 * i, h] = slab[:, 0:128]
            vs_ref[2 * i + 1, h] = slab[:, 128:256]
        if first:
            for part in range(3):
                cp_b[part].wait()
                permute_rows(wb_ref[part].astype(jnp.float32).T, wbt_ref, part * D)
            cp_ob.wait()
            permute_rows(wob_ref[...].astype(jnp.float32), wop_ref, 0)
            cp_oa.wait()
            bproj()
            bchunks(0, nb)
            oprojb(0)
            oprojb(1)
        units = [(qb, g) for qb in range(2) for g in range(G)]
        nkf = lambda qb: (qb + 1) if first else 3
        def qk(u):
            qb, g = units[u]
            _qk(g, nkf(qb), qb, base + qb * 128, ka_ref, qa_ref, s_ref, u % NS)
        def sm(u, hh):
            _softmax(hh, nkf(units[u][0]), s_ref, p_ref, u % NS, upper, umask)
        def pv(u, hh):
            qb, g = units[u]
            _pv(g, hh, nkf(qb), base + qb * 128, vs_ref, p_ref, ot_ref.at[qb], u % NS)
        def oproj(qb):
            r = slice(qb * 128, (qb + 1) * 128)
            oa = ot_ref[qb].T.astype(jnp.bfloat16)
            a = jnp.dot(oa, woa_ref[...], preferred_element_type=jnp.float32)
            o_ref[r, :] = (gate[r] * a + acc_ref[r, :]).astype(o_ref.dtype)
        qk(0)
        for u in range(len(units)):
            if u + 1 < len(units):
                qk(u + 1)
            for hh in range(4):
                sm(u, hh)
            if u >= 1:
                for hh in range(4):
                    pv(u - 1, hh)
            if u == G + 2:
                oproj(0)
        for hh in range(4):
            pv(len(units) - 1, hh)
        oproj(1)

    @pl.when(i == 0)
    def _():
        body(True)

    @pl.when(i > 0)
    def _():
        body(False)


@jax.jit
def pallas_gated_mix__sliding_block__sliding_local_dilated__prompt_kernel(
    A_x, A_wqkv, A_wo, B_x, B_wqkv, B_wo, gate_w,
):
    xa = A_x.reshape(S, D)
    gw = gate_w.reshape(1, D)
    full = lambda shape: pl.BlockSpec(shape, lambda i: (0,) * len(shape))
    out = pl.pallas_call(
        _kernel,
        grid=(S // BQ,),
        in_specs=[
            pl.BlockSpec((BQ, D), lambda i: (i, 0)),
            pl.BlockSpec(memory_space=pl.ANY), pl.BlockSpec(memory_space=pl.ANY),
            pl.BlockSpec(memory_space=pl.ANY), pl.BlockSpec(memory_space=pl.ANY), full((1, D)),
        ],
        out_specs=pl.BlockSpec((BQ, D), lambda i: (i, 0)),
        out_shape=jax.ShapeDtypeStruct((S, D), jnp.bfloat16),
        scratch_shapes=[
            pltpu.VMEM((G, S, 128), jnp.bfloat16),
            pltpu.VMEM((G, BQ, 128), jnp.float32),
            pltpu.VMEM((S // 128, H, 32, 128), jnp.bfloat16),
            pltpu.VMEM((NS, 384, 512), jnp.float32),
            pltpu.VMEM((NS, 384, 512), jnp.bfloat16),
            pltpu.VMEM((2, D, 128), jnp.float32),
            pltpu.VMEM((BQ, D), jnp.bfloat16),
            pltpu.VMEM((NT, BQ, 128), jnp.float32),
            pltpu.VMEM((NT, PADB + S, 128), jnp.float32),
            pltpu.VMEM((NT, PADB + S, 128), jnp.float32),
            pltpu.VMEM((BQ, D), jnp.bfloat16),
            pltpu.VMEM((3 * D, D), jnp.bfloat16),
            pltpu.VMEM((D, D), jnp.bfloat16),
            pltpu.VMEM((NT, D, 128), jnp.float32),
            pltpu.VMEM((BQ, D), jnp.float32),
            pltpu.VMEM((3, D, D), jnp.bfloat16),
            pltpu.VMEM((3, D, D), jnp.bfloat16),
            pltpu.VMEM((D, D), jnp.bfloat16),
            pltpu.VMEM((D, D), jnp.bfloat16),
            pltpu.SemaphoreType.DMA((8,)),
        ],
        compiler_params=pltpu.CompilerParams(
            dimension_semantics=("arbitrary",), vmem_limit_bytes=100 * 2 ** 20),
    )(xa, A_wqkv, B_wqkv, A_wo, B_wo, gw)
    return out.reshape(1, S, D)
```
